```python
import os as _os
_os.environ.setdefault("JAX_PLATFORMS", "cpu")
import jax
import jax.numpy as jnp

def _softmax(x, axis=-1):
    return jax.nn.softmax(x, axis=axis)
def _gelu(x):
    return jax.nn.gelu(x, approximate=True)
def _silu(x):
    return jax.nn.silu(x)
def _sigmoid(x):
    return jax.nn.sigmoid(x)
def _layernorm(x, axis=-1, eps=1e-5):
    m = jnp.mean(x, axis=axis, keepdims=True)
    v = jnp.var(x, axis=axis, keepdims=True)
    return (x - m) / jnp.sqrt(v + eps)
def _scatter_add(tgt, idx, src, axis=0):
    return tgt.at[idx].add(src)
def _segment_sum(src, seg, n):
    return jax.ops.segment_sum(src, seg, n)
class _Rng:
    def __init__(self, key):
        self._k = key
    def _next(self):
        self._k, sub = jax.random.split(self._k)
        return sub
    def normal(self, shape):
        return jax.random.normal(self._next(), shape, dtype=jnp.bfloat16)
    def randint(self, lo, hi, shape):
        return jax.random.randint(self._next(), shape, lo, hi, dtype=jnp.int32)
    def uniform(self, shape, lo=0.0, hi=1.0):
        return jax.random.uniform(self._next(), shape, jnp.bfloat16, lo, hi)
    def permutation(self, n):
        return jax.random.permutation(self._next(), n)


kernel_name = 'standalone__mha_softmax__near_ridge'

def setup_inputs():
    _rng = _Rng(jax.random.key(int.from_bytes(__import__("os").urandom(4), "little")))
    _w = (lambda a: (lambda t: t.astype(jnp.bfloat16) if jnp.issubdtype(t.dtype, jnp.floating) else t)(jnp.asarray(a)))
    B, H, Sq, Sk, D = 8, 32, 496, 512, 192
    return {
        "q": _w((lambda *s: _rng.normal(s) * 0.05)(B, H, Sq, D)),
        "k": _w((lambda *s: _rng.normal(s) * 3.2)(B, H, Sk, D)),
        "v": _w((lambda *s: _rng.normal(s) * 0.05)(B, H, Sk, D)),
    }

def reference(q, k, v):
    scale = q.shape[-1] ** -0.5
    scores = jnp.einsum("bhqd,bhkd->bhqk", q, k) * scale
    p = _softmax(scores, axis=-1)
    return jnp.einsum("bhqk,bhkd->bhqd", p, v)
```

```python
import functools
import jax, jax.numpy as jnp
import jax.experimental.pallas as pl
import jax.experimental.pallas.tpu as pltpu

HB = 4
MODE = "T1"

def kern(q_ref, k_ref, v_ref, o_ref, *, scale):
    for h in range(HB):
        qt = q_ref[0, h]
        kt = k_ref[0, h]
        vt = v_ref[0, h]
        if MODE == "T1":
            st = jax.lax.dot_general(kt, qt, (((0,), (0,)), ((), ())), preferred_element_type=jnp.float32) * scale
            m = jnp.max(st, axis=0, keepdims=True)
            p = jnp.exp(st - m)
            l = jnp.sum(p, axis=0, keepdims=True)
            ot = jnp.dot(vt, p.astype(jnp.bfloat16), preferred_element_type=jnp.float32)
            o_ref[0, h] = (ot / l).astype(o_ref.dtype)
        else:
            s = jax.lax.dot_general(qt, kt, (((0,), (0,)), ((), ())), preferred_element_type=jnp.float32) * scale
            m = jnp.max(s, axis=1, keepdims=True)
            p = jnp.exp(s - m)
            l = jnp.sum(p, axis=1, keepdims=True)
            p = (p / l).astype(jnp.bfloat16)
            ot = jax.lax.dot_general(vt, p, (((1,), (1,)), ((), ())), preferred_element_type=jnp.float32)
            o_ref[0, h] = ot.astype(o_ref.dtype)

@jax.jit
def pallas_standalone__mha_softmax__near_ridge_kernel(q, k, v):
    B, H, Sq, D = q.shape
    Sk = k.shape[2]
    scale = D ** -0.5
    qt = jnp.swapaxes(q, 2, 3); kt = jnp.swapaxes(k, 2, 3); vt = jnp.swapaxes(v, 2, 3)
    ot = pl.pallas_call(
        functools.partial(kern, scale=scale),
        grid=(B, H // HB),
        in_specs=[pl.BlockSpec((1, HB, D, Sq), lambda b, h: (b, h, 0, 0)),
                  pl.BlockSpec((1, HB, D, Sk), lambda b, h: (b, h, 0, 0)),
                  pl.BlockSpec((1, HB, D, Sk), lambda b, h: (b, h, 0, 0))],
        out_specs=pl.BlockSpec((1, HB, D, Sq), lambda b, h: (b, h, 0, 0)),
        out_shape=jax.ShapeDtypeStruct((B, H, D, Sq), q.dtype),
        compiler_params=pltpu.CompilerParams(dimension_semantics=("parallel", "parallel"), vmem_limit_bytes=64*1024*1024),
    )(qt, kt, vt)
    return jnp.swapaxes(ot, 2, 3)
```

```python
import functools, math
import jax, jax.numpy as jnp
import jax.experimental.pallas as pl
import jax.experimental.pallas.tpu as pltpu

HB = 8

def kern(q_ref, k_ref, v_ref, o_ref, *, c2):
    def qk(h):
        return jax.lax.dot_general(k_ref[0, h], q_ref[0, h], (((0,), (0,)), ((), ())), preferred_element_type=jnp.float32)
    def sm(st):
        m = jnp.max(st, axis=0, keepdims=True)
        p = jnp.exp2((st - m) * c2)
        l = jnp.sum(p, axis=0, keepdims=True)
        return p.astype(jnp.bfloat16), l
    def pv(h, p, l):
        ot = jnp.dot(v_ref[0, h], p, preferred_element_type=jnp.float32)
        o_ref[0, h] = (ot / l).astype(o_ref.dtype)
    st = {0: qk(0), 1: qk(1)}
    pl_ = {}
    for t in range(HB + 1):
        if t + 2 < HB:
            st[t + 2] = qk(t + 2)
        if t - 1 >= 0:
            pv(t - 1, *pl_.pop(t - 1))
        if t < HB:
            pl_[t] = sm(st.pop(t))

@jax.jit
def pallas_standalone__mha_softmax__near_ridge_kernel(q, k, v):
    B, H, Sq, D = q.shape
    Sk = k.shape[2]
    c2 = (D ** -0.5) * math.log2(math.e)
    qt = jnp.swapaxes(q, 2, 3); kt = jnp.swapaxes(k, 2, 3); vt = jnp.swapaxes(v, 2, 3)
    ot = pl.pallas_call(
        functools.partial(kern, c2=c2),
        grid=(B, H // HB),
        in_specs=[pl.BlockSpec((1, HB, D, Sq), lambda b, h: (b, h, 0, 0)),
                  pl.BlockSpec((1, HB, D, Sk), lambda b, h: (b, h, 0, 0)),
                  pl.BlockSpec((1, HB, D, Sk), lambda b, h: (b, h, 0, 0))],
        out_specs=pl.BlockSpec((1, HB, D, Sq), lambda b, h: (b, h, 0, 0)),
        out_shape=jax.ShapeDtypeStruct((B, H, D, Sq), q.dtype),
        compiler_params=pltpu.CompilerParams(dimension_semantics=("parallel", "parallel"), vmem_limit_bytes=96*1024*1024),
    )(qt, kt, vt)
    return jnp.swapaxes(ot, 2, 3)
```
